```python
import os as _os
_os.environ.setdefault('JAX_PLATFORMS', 'cpu')
import jax
import jax.numpy as jnp

def _softmax(x, axis=-1):
    return jax.nn.softmax(x, axis=axis)

def _gelu(x):
    return jax.nn.gelu(x, approximate=True)

def _silu(x):
    return jax.nn.silu(x)

def _sigmoid(x):
    return jax.nn.sigmoid(x)

def _layernorm(x, axis=-1, eps=1e-05):
    m = jnp.mean(x, axis=axis, keepdims=True)
    v = jnp.var(x, axis=axis, keepdims=True)
    return (x - m) / jnp.sqrt(v + eps)

def _scatter_add(tgt, idx, src, axis=0):
    return tgt.at[idx].add(src)

def _segment_sum(src, seg, n):
    return jax.ops.segment_sum(src, seg, n)

class _Rng:

    def __init__(self, key):
        self._k = key

    def _next(self):
        self._k, sub = jax.random.split(self._k)
        return sub

    def normal(self, shape):
        return jax.random.normal(self._next(), shape, dtype=jnp.bfloat16)

    def randint(self, lo, hi, shape):
        return jax.random.randint(self._next(), shape, lo, hi, dtype=jnp.int32)

    def uniform(self, shape, lo=0.0, hi=1.0):
        return jax.random.uniform(self._next(), shape, jnp.bfloat16, lo, hi)

    def permutation(self, n):
        return jax.random.permutation(self._next(), n)
kernel_name = 'gated_mix__memory_aug_recurrent_mem_tr__glu_gated_geglu__prompt'

def setup_inputs():
    _rng = _Rng(jax.random.key(int.from_bytes(__import__("os").urandom(4), "little")))
    _w = lambda a: (lambda t: t.astype(jnp.bfloat16) if jnp.issubdtype(t.dtype, jnp.floating) else t)(jnp.asarray(a))

    def _A_setup():
        B, S, Dm = (1, 2048, 640)
        H, Dh = (32, 128)
        M, seg = (8, 32)
        seg = min(seg, S)
        S = S // seg * seg
        return {'x': _w((lambda *s: _rng.normal(s) * 0.05)(B, S, Dm)), 'mem0': _w((lambda *s: _rng.normal(s) * 0.4)(B, M, Dm)), 'Wq': _w((lambda *s: _rng.normal(s) * 3.2)(Dm, H, Dh) * Dm ** (-0.5)), 'Wk': _w((lambda *s: _rng.normal(s) * 3.2)(Dm, H, Dh) * Dm ** (-0.5)), 'Wv': _w((lambda *s: _rng.normal(s) * 0.4)(Dm, H, Dh) * Dm ** (-0.5)), 'Wo': _w((lambda *s: _rng.normal(s) * 0.4)(H, Dh, Dm) * (H * Dh) ** (-0.5)), 'seg_len': seg}
    _A_in = _A_setup()

    def _B_setup():
        B, S, Dm, Df = (1, 2048, 640, 1728)
        return {'x': _w((lambda *s: _rng.normal(s) * 0.05)(B, S, Dm)), 'w_gate': _w((lambda *s: _rng.normal(s) * 1.6)(Dm, Df) * Dm ** (-0.5)), 'w_up': _w((lambda *s: _rng.normal(s) * 1.6)(Dm, Df) * Dm ** (-0.5)), 'w_down': _w((lambda *s: _rng.normal(s) * 1.6)(Df, Dm) * Df ** (-0.5))}
    _B_in = _B_setup()
    return {'A_x': _A_in['x'], 'A_mem0': _A_in['mem0'], 'A_Wq': _A_in['Wq'], 'A_Wk': _A_in['Wk'], 'A_Wv': _A_in['Wv'], 'A_Wo': _A_in['Wo'], 'A_seg_len': _A_in['seg_len'], 'B_x': _B_in['x'], 'B_w_gate': _B_in['w_gate'], 'B_w_up': _B_in['w_up'], 'B_w_down': _B_in['w_down'], 'gate_w': _w((lambda *s: _rng.normal(s) * 0.05)(640) * 16.0)}

def reference(A_x, A_mem0, A_Wq, A_Wk, A_Wv, A_Wo, A_seg_len, B_x, B_w_gate, B_w_up, B_w_down, gate_w):

    def _A_ref(x, mem0, Wq, Wk, Wv, Wo, seg_len):
        B, S, Dm = x.shape
        H, Dh = (Wq.shape[1], Wq.shape[2])
        M = mem0.shape[1]
        scale = Dh ** (-0.5)
        n_seg = S // seg_len
        L = M + seg_len
        idx = jnp.arange(L)
        mask = (idx[:, None] < M) | (idx[:, None] >= idx[None, :])
        mem = mem0
        outs = []
        for s in range(n_seg):
            xs = x[:, s * seg_len:(s + 1) * seg_len, :].copy()
            h = jnp.concatenate([mem, xs], axis=1)
            q = jnp.einsum('btd,dhe->bhte', h, Wq)
            k = jnp.einsum('btd,dhe->bhte', h, Wk)
            v = jnp.einsum('btd,dhe->bhte', h, Wv)
            scores = jnp.einsum('bhqe,bhke->bhqk', q, k) * scale
            scores = jnp.where(mask[None, None], scores, -1000000000.0)
            p = _softmax(scores, axis=-1)
            o = jnp.einsum('bhqk,bhke->bhqe', p, v)
            o = jnp.einsum('bhte,hed->btd', o, Wo)
            mem = o[:, :M, :].copy()
            outs.append(o[:, M:, :])
        return jnp.concatenate(outs, axis=1)

    def _B_ref(x, w_gate, w_up, w_down):
        g = jnp.einsum('bsd,df->bsf', x, w_gate)
        u = jnp.einsum('bsd,df->bsf', x, w_up)
        h = _gelu(g) * u
        return jnp.einsum('bsf,fd->bsd', h, w_down)
    x = A_x
    g = _sigmoid((x * gate_w).sum(-1, keepdims=True))
    a = _A_ref(x, A_mem0, A_Wq, A_Wk, A_Wv, A_Wo, A_seg_len)
    b = _B_ref(x, B_w_gate, B_w_up, B_w_down)
    return g * a + (1 - g) * b
```

```python
import functools

import jax
import jax.numpy as jnp
import numpy as np
import jax.experimental.pallas as pl
import jax.experimental.pallas.tpu as pltpu

NT = (((1,), (1,)), ((), ()))
F32 = jnp.float32
BF16 = jnp.bfloat16
HG = 4
RB = 64
PRE = 8


def _gelu(x):
    c = float(np.sqrt(2.0 / np.pi))
    return 0.5 * x * (1.0 + jnp.tanh(c * (x + 0.044715 * (x * x * x))))


def _kernel(ax_h, mem0_ref, wq_h, wk_h, wv_h, wo_h, wg_h, wu_h, wd_h, gw_ref, out_ref,
            ax, stage, wqkv, wo, wg, wu, wd, tok, otok, abuf, sems,
            *, S, Dm, H, Dh, M, SEG, DF):
    NP = S // (2 * SEG)
    scale = float(Dh) ** -0.5
    HW = H // 2
    c_wg = pltpu.make_async_copy(wg_h, wg, sems.at[1])
    c_wu = pltpu.make_async_copy(wu_h, wu, sems.at[2])
    c_wd = pltpu.make_async_copy(wd_h, wd, sems.at[3])
    c_ax = pltpu.make_async_copy(ax_h, ax.at[pl.ds(0, S)], sems.at[4])
    c_w = [pltpu.make_async_copy(w.bitcast(jnp.uint32), stage.at[i], sems.at[5 + i])
           for i, w in enumerate((wq_h, wk_h, wv_h))]
    c_wo = pltpu.make_async_copy(wo_h, wo, sems.at[8])
    for c in (c_ax, c_wg, c_wu, c_wd, *c_w, c_wo):
        c.start()

    def ffn(r0, n=2 * SEG):
        xb = ax[pl.ds(r0, n), :]
        g = jax.lax.dot_general(xb, wg[...], NT, preferred_element_type=F32)
        u = jax.lax.dot_general(xb, wu[...], NT, preferred_element_type=F32)
        hh = (_gelu(g) * u).astype(BF16)
        return jnp.dot(hh, wd[...], preferred_element_type=F32)

    def gate(r0):
        xa = ax[pl.ds(r0, 2 * SEG), :].astype(F32)
        z = jnp.sum(xa * gw_ref[...].astype(F32), axis=-1, keepdims=True)
        return 1.0 / (1.0 + jnp.exp(-z))

    c_ax.wait(); c_wg.wait(); c_wu.wait(); c_wd.wait()

    def pre_body(i, c):
        r0 = pl.multiple_of(i * 4 * SEG, 4 * SEG)
        out_ref[pl.ds(r0, 4 * SEG), :] = ffn(r0, 4 * SEG).astype(out_ref.dtype)
        return c
    lax_fori(0, PRE // 2, pre_body)

    ax[pl.ds(S, 2 * SEG), :] = jnp.zeros((2 * SEG, Dm), BF16)
    for i in range(3):
        c_w[i].wait()

        def rl_body(b, c, i=i):
            sv = stage
            d0 = pl.multiple_of(b * RB, RB)
            for j in range(HW):
                w = sv[i, b, pl.ds(j, RB, stride=HW), :]
                lo = pltpu.bitcast(w << 16, F32).astype(BF16)
                hi = pltpu.bitcast(w & jnp.uint32(0xFFFF0000), F32).astype(BF16)
                wqkv[pl.ds(d0, RB), pl.ds(((2 * j) * 3 + i) * Dh, Dh)] = lo
                wqkv[pl.ds(d0, RB), pl.ds(((2 * j + 1) * 3 + i) * Dh, Dh)] = hi
            return c
        lax_fori(0, Dm // RB, rl_body)
    c_wo.wait()

    GW = HG * 3 * Dh
    NG = H // HG
    for g in range(NG):
        tok[pl.ds(2 * SEG, SEG), pl.ds(g * GW, GW)] = jnp.dot(
            ax[pl.ds(0, SEG), :], wqkv[:, pl.ds(g * GW, GW)], preferred_element_type=F32)
    otok[...] = jnp.zeros(otok.shape, F32)

    L = M + SEG
    LP = L + 8
    row = jax.lax.broadcasted_iota(jnp.int32, (LP, LP), 0)
    col = jax.lax.broadcasted_iota(jnp.int32, (LP, LP), 1)
    mask = ((row < M) | (row >= col)) & (col < L)
    zpad = jnp.zeros((8, Dh), F32)

    def step(mem, r0, odd):
        if not odd:
            nt, x0, t0 = 24, r0 + SEG, SEG
        else:
            nt, x0, t0 = 40, r0 + SEG + 24, SEG + 24
        if not odd:
            xt = ax[pl.ds(pl.multiple_of(x0, 16), 32), :].astype(F32)[:24]
        else:
            xt = ax[pl.ds(pl.multiple_of(x0 - 8, 16), 48), :].astype(F32)[8:]
        lhs = jnp.concatenate([mem, xt], axis=0).astype(BF16)
        s0 = SEG if odd else 0
        def proj(g):
            cs = pl.ds(g * GW, GW)
            if not odd:
                cur = tok[pl.ds(2 * SEG, SEG), cs]
            else:
                old = tok[pl.ds(SEG, 24), cs]
            pr = jnp.dot(lhs, wqkv[:, cs], preferred_element_type=F32)
            if odd:
                cur = jnp.concatenate([old, pr[M:M + 8]], axis=0)
                tok[pl.ds(2 * SEG, SEG), cs] = pr[M + 8:]
            else:
                tok[pl.ds(SEG, 24), cs] = pr[M:]
            return jnp.concatenate(
                [pr[:M], cur, jnp.zeros((8, GW), F32)], axis=0).astype(BF16)

        def scores(qkv):
            return [jax.lax.dot_general(
                qkv[:, hh * 3 * Dh:(hh * 3 + 1) * Dh], qkv[:, (hh * 3 + 1) * Dh:(hh * 3 + 2) * Dh],
                NT, preferred_element_type=F32) for hh in range(HG)]

        def soft(scs):
            ps = []
            for sc in scs:
                sc = jnp.where(mask, sc * scale, -1e9)
                e = jnp.exp(sc - jnp.max(sc, axis=-1, keepdims=True))
                ps.append((e / jnp.sum(e, axis=-1, keepdims=True)).astype(BF16))
            return ps

        def pv(ps, qkv):
            return jnp.concatenate(
                [jnp.dot(ps[hh], qkv[:, (hh * 3 + 2) * Dh:(hh * 3 + 3) * Dh],
                         preferred_element_type=F32) for hh in range(HG)], axis=1)

        def outp(g, o):
            oc = pl.ds(g * HG * Dh, HG * Dh)
            if not odd:
                ol = jnp.concatenate([o[:M], otok[pl.ds(0, 8), oc], o[M:M + 16]], axis=0)
                otok[pl.ds(8, 16), oc] = o[M + 16:L]
            else:
                ol = jnp.concatenate([o[:M], otok[pl.ds(8, 16), oc], o[M:M + 24]], axis=0)
                otok[pl.ds(0, 8), oc] = o[L - 8:L]
            return jnp.dot(ol.astype(BF16), wo[oc, :], preferred_element_type=F32)

        acc = None
        Q, SC, P, O = {}, {}, {}, {}
        for t in range(NG + 4):
            if t < NG:
                Q[t] = proj(t)
            if 0 <= t - 1 < NG:
                SC[t - 1] = scores(Q[t - 1])
            if 0 <= t - 2 < NG:
                P[t - 2] = soft(SC[t - 2])
            if 0 <= t - 3 < NG:
                O[t - 3] = pv(P[t - 3], Q[t - 3])
            if 0 <= t - 4 < NG:
                d = outp(t - 4, O[t - 4])
                acc = d if acc is None else acc + d
        a0 = r0 + 24 if odd else r0
        abuf[pl.ds(pl.multiple_of(a0, 8), nt), :] = acc[M:]
        return acc[:M]

    def combine(r0, b):
        g = gate(r0)
        a = abuf[pl.ds(pl.multiple_of(r0 + 8, 8), 2 * SEG), :]
        out_ref[pl.ds(r0, 2 * SEG), :] = (g * a + (1.0 - g) * b).astype(out_ref.dtype)

    def pair(j, mem, with_ffn):
        r0 = pl.multiple_of(j * 2 * SEG, 2 * SEG)
        mem = step(mem, r0, False)
        mem = step(mem, r0, True)
        if with_ffn:
            rp = pl.multiple_of(r0 - 2 * SEG, 2 * SEG)
            combine(rp, ffn(rp))
        return mem

    mem = mem0_ref[...].astype(F32)
    mem = jax.lax.fori_loop(0, PRE + 1, lambda j, m: pair(j, m, False), mem)
    mem = jax.lax.fori_loop(PRE + 1, NP, lambda j, m: pair(j, m, True), mem)

    abuf[pl.ds(S, 8), :] = jnp.dot(otok[pl.ds(0, 16), :].astype(BF16), wo[...],
                                   preferred_element_type=F32)[:8]
    combine(S - 2 * SEG, ffn(S - 2 * SEG))

    def post_body(i, c):
        r0 = pl.multiple_of(i * 2 * SEG, 2 * SEG)
        combine(r0, out_ref[pl.ds(r0, 2 * SEG), :].astype(F32))
        return c
    lax_fori(0, PRE, post_body)


def lax_fori(lo, hi, body):
    jax.lax.fori_loop(lo, hi, body, 0)


@jax.jit
def pallas_gated_mix__memory_aug_recurrent_mem_tr__glu_gated_geglu__prompt_kernel(
    A_x, A_mem0, A_Wq, A_Wk, A_Wv, A_Wo, A_seg_len, B_x, B_w_gate, B_w_up, B_w_down, gate_w,
):
    B, S, Dm = A_x.shape
    _, H, Dh = A_Wq.shape
    M = A_mem0.shape[1]
    DF = B_w_gate.shape[1]
    SEG = 32
    assert B == 1 and M == 8 and S % (2 * SEG) == 0
    any_spec = pl.BlockSpec(memory_space=pl.ANY)
    vmem = pl.BlockSpec(memory_space=pltpu.VMEM)
    out = pl.pallas_call(
        functools.partial(_kernel, S=S, Dm=Dm, H=H, Dh=Dh, M=M, SEG=SEG, DF=DF),
        out_shape=jax.ShapeDtypeStruct((S, Dm), A_x.dtype),
        in_specs=[any_spec, vmem, any_spec, any_spec, any_spec, any_spec,
                  any_spec, any_spec, any_spec, vmem],
        out_specs=vmem,
        scratch_shapes=[
            pltpu.VMEM((S + 2 * SEG, Dm), BF16),
            pltpu.VMEM((3, Dm // RB, RB * H // 2, Dh), jnp.uint32),
            pltpu.VMEM((Dm, 3 * H * Dh), BF16),
            pltpu.VMEM((H * Dh, Dm), BF16),
            pltpu.VMEM((DF, Dm), BF16),
            pltpu.VMEM((DF, Dm), BF16),
            pltpu.VMEM((DF, Dm), BF16),
            pltpu.VMEM((3 * SEG, 3 * H * Dh), F32),
            pltpu.VMEM((8 + 2 * SEG, H * Dh), F32),
            pltpu.VMEM((S + 8, Dm), F32),
            pltpu.SemaphoreType.DMA((9,)),
        ],
        compiler_params=pltpu.CompilerParams(vmem_limit_bytes=110 * 2**20),
    )(A_x.reshape(S, Dm), A_mem0.reshape(M, Dm), A_Wq.reshape(Dm // RB, RB * H, Dh),
      A_Wk.reshape(Dm // RB, RB * H, Dh), A_Wv.reshape(Dm // RB, RB * H, Dh), A_Wo.reshape(H * Dh, Dm),
      B_w_gate.T, B_w_up.T, B_w_down, gate_w.reshape(1, Dm))
    return out.reshape(B, S, Dm)
```
